```python
import jax
import jax.numpy as jnp

def _softmax(x, axis=-1):
    return jax.nn.softmax(x, axis=axis)
def _gelu(x):
    return jax.nn.gelu(x, approximate=True)
def _silu(x):
    return jax.nn.silu(x)
def _sigmoid(x):
    return jax.nn.sigmoid(x)
def _layernorm(x, axis=-1, eps=1e-5):
    m = jnp.mean(x, axis=axis, keepdims=True)
    v = jnp.var(x, axis=axis, keepdims=True)
    return (x - m) / jnp.sqrt(v + eps)
def _scatter_add(tgt, idx, src, axis=0):
    return tgt.at[idx].add(src)
def _segment_sum(src, seg, n):
    return jax.ops.segment_sum(src, seg, n)
class _Rng:
    def __init__(self, key):
        self._k = key
    def _next(self):
        self._k, sub = jax.random.split(self._k)
        return sub
    def normal(self, shape):
        return jax.random.normal(self._next(), shape, dtype=jnp.bfloat16)
    def randint(self, lo, hi, shape):
        return jax.random.randint(self._next(), shape, lo, hi, dtype=jnp.int32)
    def uniform(self, shape, lo=0.0, hi=1.0):
        return jax.random.uniform(self._next(), shape, jnp.bfloat16, lo, hi)
    def permutation(self, n):
        return jax.random.permutation(self._next(), n)


kernel_name = 'recurrent_scan__compressed_kv_cla__moe_arch_mod__decode'

def setup_inputs():
    _rng = _Rng(jax.random.key(int.from_bytes(__import__("os").urandom(4), "little")))
    _w = (lambda a: (lambda t: t.astype(jnp.bfloat16) if jnp.issubdtype(t.dtype, jnp.floating) else t)(jnp.asarray(a)))
    def _A_setup():
        B, H, Sq, Sk, D, M = 4, 32, 1, 4096, 128, 576
        Dc = 4 * D
        return {
            "x": _w((lambda *s: _rng.normal(s) * 0.05)(B, Sq, M)),
            "c_kv": _w((lambda *s: _rng.normal(s) * 0.05)(B, Sk, Dc)),
            "w_q": _w((lambda *s: _rng.normal(s) * 0.05)(M, H, D) * (M ** -0.5)),
            "w_uk": _w((lambda *s: _rng.normal(s) * 0.05)(Dc, H, D) * (Dc ** -0.5)),
            "w_uv": _w((lambda *s: _rng.normal(s) * 0.05)(Dc, H, D) * (Dc ** -0.5)),
            "w_o": _w((lambda *s: _rng.normal(s) * 0.05)(H, D, M) * ((H * D) ** -0.5)),
        }
    _A_in = _A_setup()

    def _B_setup():
        B, S, D, F, C = 4, 1, 576, 4608, 1
        return {
            "x": _w((lambda *s: _rng.normal(s) * 0.05)(B, S, D)),
            "w_r": _w((lambda *s: _rng.normal(s) * 0.05)(D)),
            "w_gate": _w((lambda *s: _rng.normal(s) * 0.05)(D, F)),
            "w_up": _w((lambda *s: _rng.normal(s) * 0.05)(D, F)),
            "w_down": _w((lambda *s: _rng.normal(s) * 0.05)(F, D)),
        }
    _B_in = _B_setup()

    return {
        "A_x": _A_in["x"],
        "A_c_kv": _A_in["c_kv"],
        "A_w_q": _A_in["w_q"],
        "A_w_uk": _A_in["w_uk"],
        "A_w_uv": _A_in["w_uv"],
        "A_w_o": _A_in["w_o"],
        "B_x": _B_in["x"],
        "B_w_r": _B_in["w_r"],
        "B_w_gate": _B_in["w_gate"],
        "B_w_up": _B_in["w_up"],
        "B_w_down": _B_in["w_down"],
    }

def reference(A_x, A_c_kv, A_w_q, A_w_uk, A_w_uv, A_w_o, B_x, B_w_r, B_w_gate, B_w_up, B_w_down):
    def _A_ref(x, c_kv, w_q, w_uk, w_uv, w_o):
        B, Sq, M = x.shape[0], x.shape[1], x.shape[2]
        Sk = c_kv.shape[1]
        H, D = w_q.shape[1], w_q.shape[2]
        q = jnp.einsum("bqm,mhd->bhqd", x, w_q)
        k = jnp.einsum("bkc,chd->bhkd", c_kv, w_uk)
        v = jnp.einsum("bkc,chd->bhkd", c_kv, w_uv)
        scores = jnp.einsum("bhqd,bhkd->bhqk", q, k) * (D ** -0.5)
        off = Sk - Sq
        qi = jnp.arange(Sq)[:, None]
        kj = jnp.arange(Sk)[None, :]
        cmask = kj <= (qi + off)
        scores = jnp.where(cmask[None, None], scores, -1e9)
        p = _softmax(scores, axis=-1)
        ctx = jnp.einsum("bhqk,bhkd->bhqd", p, v)
        return jnp.einsum("bhqd,hdm->bqm", ctx, w_o)

    def _B_ref(x, w_r, w_gate, w_up, w_down):
        B, S, D = x.shape
        C = 1
        r = x @ w_r
        idx = jnp.argsort(-r, axis=-1)[:, :C]
        idx_e = jnp.repeat(idx.reshape(B, C, 1), D, axis=2)
        x_sel = jnp.take_along_axis(x, idx_e, axis=1)
        g = _silu(x_sel @ w_gate)
        u = x_sel @ w_up
        y = (g * u) @ w_down
        r_sel = _sigmoid(jnp.take_along_axis(r, idx, axis=1))
        y = y * r_sel.reshape(B, C, 1)
        b_off = (jnp.arange(B) * S).reshape(B, 1)
        flat_idx = (idx + b_off).reshape(B * C)
        zero = (x * 0.0).reshape(B * S, D)
        upd = _scatter_add(zero, flat_idx, y.reshape(B * C, D), axis=0)
        return x + upd.reshape(B, S, D)

    x = A_x
    xn = _layernorm(x, axis=-1)
    s = _A_ref(xn, A_c_kv, A_w_q, A_w_uk, A_w_uv, A_w_o)
    g = _silu(_B_ref(xn, B_w_r, B_w_gate, B_w_up, B_w_down))
    return x + s * g
```

```python
import functools
import jax
import jax.numpy as jnp
from jax import lax
import jax.experimental.pallas as pl
import jax.experimental.pallas.tpu as pltpu

B, H, SK, D, M = 4, 32, 4096, 128, 576
DC = 512
F = 4608
HH = 16
KC = 512
FC = 512
WO_CHUNKS = (8, 8, 8, 4, 2, 1, 1)

f32 = jnp.float32
bf16 = jnp.bfloat16
NN = (((1,), (0,)), ((), ()))
NT = (((1,), (1,)), ((), ()))


def _dot(a, b, dims):
    return lax.dot_general(a, b, dims, preferred_element_type=f32)


def _kernel(x_hbm, wr_hbm, ckv_hbm, wq_hbm, wuk_hbm, wuv_hbm, wo_hbm, wg_hbm, wu_hbm, wd_hbm,
            o_hbm,
            x_v, wr_v, ckv_v, wq_v, wuk_v, wuv_v, wo_v, wg_v, wu_v, wd_v, o_v,
            rep_v, xexp_v, qabs_v, s_v, p_v, ctxc_v, ctx_v, h_v, sems):
    sem_id = [0]

    def cp(src, dst):
        c = pltpu.make_async_copy(src, dst, sems.at[sem_id[0]])
        sem_id[0] += 1
        return c

    c_x = cp(x_hbm, x_v)
    c_wr = cp(wr_hbm, wr_v)
    c_wq = cp(wq_hbm, wq_v)
    c_wuk = cp(wuk_hbm, wuk_v)
    ckv_sem0 = sem_id[0]
    c_ckv = [cp(ckv_hbm.at[b], ckv_v.at[b]) for b in range(B)]
    c_wuv = cp(wuv_hbm, wuv_v)
    c_wg = cp(wg_hbm, wg_v)
    c_wu = cp(wu_hbm, wu_v)
    c_wd = cp(wd_hbm, wd_v)
    c_wo = []
    h0 = 0
    for n in WO_CHUNKS:
        c_wo.append(cp(wo_hbm.at[pl.ds(h0, n)], wo_v.at[pl.ds(h0, n)]))
        h0 += n
    c_out = cp(o_v, o_hbm)
    for c in [c_x, c_wr, c_wq, c_wuk] + c_ckv + [c_wuv, c_wg, c_wu, c_wd] + c_wo:
        c.start()

    def rep_body(t, carry):
        row = lax.broadcasted_iota(jnp.int32, (128, 256), 0)
        col = lax.broadcasted_iota(jnp.int32, (128, 256), 1) + t * 256
        rep_v[t] = jnp.where((col >> 4) == row, 1.0, 0.0).astype(bf16)
        return carry
    lax.fori_loop(0, 8, rep_body, 0)

    def head_mask(width):
        row = lax.broadcasted_iota(jnp.int32, (B * HH, width), 0)
        col = lax.broadcasted_iota(jnp.int32, (B * HH, width), 1)
        return (row & (HH - 1)) == (col & (HH - 1))

    c_x.wait()
    c_wr.wait()
    x = x_v[...].astype(f32)
    mu = jnp.mean(x, axis=-1, keepdims=True)
    xc = x - mu
    var = jnp.mean(xc * xc, axis=-1, keepdims=True)
    xn_b = (xc / jnp.sqrt(var + 1e-5)).astype(bf16)
    xn = xn_b.astype(f32)
    wr = wr_v[...].astype(f32).reshape(1, M)
    r = jnp.sum(xn * wr, axis=-1, keepdims=True)
    r_sel = jax.nn.sigmoid(r)

    mask256 = head_mask(256)
    for j in range(5):
        w = 128 if j < 4 else 64
        xj = xn_b[:, 128 * j:128 * j + w]
        for t in range(w // 16):
            xr = _dot(xj, rep_v[t, 0:w, :], NN)
            xb = jnp.concatenate(
                [jnp.broadcast_to(xr[b:b + 1, :], (HH, 256)) for b in range(B)], axis=0)
            xexp_v[8 * j + t] = jnp.where(mask256, xb, 0.0).astype(bf16)

    c_wq.wait()

    def q_body(t, carry):
        q0, q1 = carry
        l = xexp_v[t]
        m0 = pl.multiple_of(t * 16, 16)
        w0 = wq_v[pl.ds(m0, 16), 0:HH, :].reshape(256, D)
        w1 = wq_v[pl.ds(m0, 16), HH:H, :].reshape(256, D)
        return q0 + _dot(l, w0, NN), q1 + _dot(l, w1, NN)
    zq = jnp.zeros((B * HH, D), f32)
    q0, q1 = lax.fori_loop(0, 36, q_body, (zq, zq), unroll=4)
    scale = D ** -0.5
    qs = [(q0 * scale).astype(bf16), (q1 * scale).astype(bf16)]

    c_wuk.wait()

    def qa_body(j, carry):
        for half in range(2):
            acc = jnp.zeros((B * HH, 128), f32)
            for t in range(8):
                c0 = pl.multiple_of(j * 128 + t * 16, 16)
                w = wuk_v[pl.ds(c0, 16), half * HH:(half + 1) * HH, :].reshape(256, D)
                rr = _dot(qs[half], w, NT)
                rm = jnp.where(mask256, rr, 0.0).astype(bf16)
                acc = acc + _dot(rm, rep_v[t], NT)
            accb = acc.astype(bf16)
            for b in range(B):
                qabs_v[j, b, half * HH:(half + 1) * HH, :] = accb[b * HH:(b + 1) * HH, :]
        return carry
    lax.fori_loop(0, 4, qa_body, 0)

    def attn_body(b, carry):
        pltpu.make_async_copy(ckv_hbm.at[b], ckv_v.at[b], sems.at[ckv_sem0 + b]).wait()
        qa = jnp.concatenate([qabs_v[j, b] for j in range(4)], axis=1)

        def s_body(i, mx):
            k0 = pl.multiple_of(i * KC, KC)
            s = _dot(qa, ckv_v[b, pl.ds(k0, KC), :], NT)
            s_v[i] = s
            m = s[:, 0:128]
            for u in range(1, KC // 128):
                m = jnp.maximum(m, s[:, u * 128:(u + 1) * 128])
            return jnp.maximum(mx, m)
        mx = lax.fori_loop(0, SK // KC, s_body, jnp.full((H, 128), -jnp.inf, f32))
        mrow = jnp.max(mx, axis=-1, keepdims=True)

        def pv_body(i, carry2):
            acc, ls = carry2
            k0 = pl.multiple_of(i * KC, KC)
            p = jnp.exp(s_v[i] - mrow)
            for u in range(KC // 128):
                ls = ls + p[:, u * 128:(u + 1) * 128]
            acc = acc + _dot(p.astype(bf16), ckv_v[b, pl.ds(k0, KC), :], NN)
            return acc, ls
        acc, ls = lax.fori_loop(0, SK // KC, pv_body,
                                (jnp.zeros((H, DC), f32), jnp.zeros((H, 128), f32)))
        l = jnp.sum(ls, axis=-1, keepdims=True)
        cc = (acc / l).astype(bf16)
        for j in range(4):
            ctxc_v[j, b] = cc[:, j * 128:(j + 1) * 128]
        return carry
    lax.fori_loop(0, B, attn_body, 0)

    c_wuv.wait()

    def v_body(j, carry):
        out = []
        for half in range(2):
            acc = carry[half]
            l = jnp.concatenate(
                [ctxc_v[j, b, half * HH:(half + 1) * HH, :] for b in range(B)], axis=0)
            for t in range(8):
                c0 = pl.multiple_of(j * 128 + t * 16, 16)
                lr = _dot(l, rep_v[t], NN)
                le = jnp.where(mask256, lr, 0.0).astype(bf16)
                w = wuv_v[pl.ds(c0, 16), half * HH:(half + 1) * HH, :].reshape(256, D)
                acc = acc + _dot(le, w, NN)
            out.append(acc)
        return tuple(out)
    ctx0, ctx1 = lax.fori_loop(0, 4, v_body, (zq, zq))
    ctx_v[0:B * HH, :] = ctx0
    ctx_v[B * HH:2 * B * HH, :] = ctx1

    c_wg.wait()

    def g_body(i, carry):
        f0 = pl.multiple_of(i * FC, FC)
        g = _dot(xn_b, wg_v[:, pl.ds(f0, FC)], NN)
        h_v[i] = g * jax.nn.sigmoid(g)
        return carry
    lax.fori_loop(0, F // FC, g_body, 0)
    c_wu.wait()

    def u_body(i, carry):
        f0 = pl.multiple_of(i * FC, FC)
        h_v[i] = h_v[i] * _dot(xn_b, wu_v[:, pl.ds(f0, FC)], NN)
        return carry
    lax.fori_loop(0, F // FC, u_body, 0)
    c_wd.wait()

    def d_body(i, y):
        f0 = pl.multiple_of(i * FC, FC)
        return y + _dot(h_v[i].astype(bf16), wd_v[:, pl.ds(f0, FC)], NT)
    y = lax.fori_loop(0, F // FC, d_body, jnp.zeros((B, M), f32))
    z = xn + y * r_sel
    gate = z * jax.nn.sigmoid(z)

    def o_head(h, acc):
        row0 = (h // HH) * (B * HH) + (h % HH)
        l = ctx_v[pl.ds(row0, B, stride=HH), :].astype(bf16)
        return acc + _dot(l, wo_v[h], NT)
    s = jnp.zeros((B, M), f32)
    h0 = 0
    for n, c in zip(WO_CHUNKS, c_wo):
        c.wait()
        if n == 1:
            s = o_head(h0, s)
        else:
            s = lax.fori_loop(h0, h0 + n, o_head, s)
        h0 += n

    o_v[...] = (x + s * gate).astype(bf16)
    c_out.start()
    c_out.wait()


@jax.jit
def pallas_recurrent_scan__compressed_kv_cla__moe_arch_mod__decode_kernel(A_x, A_c_kv, A_w_q, A_w_uk, A_w_uv, A_w_o, B_x, B_w_r, B_w_gate, B_w_up, B_w_down):
    x = A_x.reshape(B, M)
    wo_t = jnp.transpose(A_w_o, (0, 2, 1))
    wd_t = B_w_down.T
    any_spec = pl.BlockSpec(memory_space=pl.ANY)
    nsem = 4 + B + 4 + len(WO_CHUNKS) + 1
    out = pl.pallas_call(
        _kernel,
        out_shape=jax.ShapeDtypeStruct((B, M), bf16),
        in_specs=[any_spec] * 10,
        out_specs=any_spec,
        scratch_shapes=[
            pltpu.VMEM((B, M), bf16),
            pltpu.VMEM((M,), bf16),
            pltpu.VMEM((B, SK, DC), bf16),
            pltpu.VMEM((M, H, D), bf16),
            pltpu.VMEM((DC, H, D), bf16),
            pltpu.VMEM((DC, H, D), bf16),
            pltpu.VMEM((H, M, D), bf16),
            pltpu.VMEM((M, F), bf16),
            pltpu.VMEM((M, F), bf16),
            pltpu.VMEM((M, F), bf16),
            pltpu.VMEM((B, M), bf16),
            pltpu.VMEM((8, 128, 256), bf16),
            pltpu.VMEM((36, B * HH, 256), bf16),
            pltpu.VMEM((4, B, H, 128), bf16),
            pltpu.VMEM((SK // KC, H, KC), f32),
            pltpu.VMEM((8, 128), f32),
            pltpu.VMEM((4, B, H, 128), bf16),
            pltpu.VMEM((2 * B * HH, D), f32),
            pltpu.VMEM((F // FC, B, FC), f32),
            pltpu.SemaphoreType.DMA((nsem,)),
        ],
        compiler_params=pltpu.CompilerParams(
            vmem_limit_bytes=100 * 1024 * 1024,
            disable_semaphore_checks=True,
        ),
    )(x, B_w_r, A_c_kv, A_w_q, A_w_uk, A_w_uv, wo_t, B_w_gate, B_w_up, wd_t)
    return out.reshape(B, 1, M)
```

```python
import functools
import jax
import jax.numpy as jnp
from jax import lax
import jax.experimental.pallas as pl
import jax.experimental.pallas.tpu as pltpu

B, H, SK, D, M = 4, 32, 4096, 128, 576
DC = 512
F = 4608
HH = 16

f32 = jnp.float32
bf16 = jnp.bfloat16
NN = (((1,), (0,)), ((), ()))
NT = (((1,), (1,)), ((), ()))


def _dot(a, b, dims):
    return lax.dot_general(a, b, dims, preferred_element_type=f32)


def make(KC=512, FC=512, NS=10, NSLOT=4, WO_CHUNKS=(8, 6, 4, 2, 1, 1), WD_CHUNKS=(3, 3, 3), skip=(), dsc=True, dbc=False, MS=512):
  assert NS + sum(WO_CHUNKS) == H and sum(WD_CHUNKS) == F // FC
  def _kernel(x_hbm, wr_hbm, ckv_hbm, wq_hbm, wuk_hbm, wuv_hbm, wo_hbm, wg_hbm, wu_hbm, wd_hbm,
            o_hbm,
            x_v, wr_v, ckv_v, wq_v, wuk_v, wuv_v, wo_v, wg_v, wu_v, wd_v, o_v,
            rep_v, xexp_v, qabs_v, s_v, ctxo_v, ctxc_v, xg_v, h_v, stage_s, sems, hsems, ssems):
    sem_id = [0]

    def cp(src, dst):
        c = pltpu.make_async_copy(src, dst, sems.at[sem_id[0]])
        sem_id[0] += 1
        return c

    def h2s(j):
        return pltpu.make_async_copy(wo_hbm.at[j], stage_s.at[j % NSLOT], hsems.at[j % NSLOT])

    def s2v(j):
        return pltpu.make_async_copy(stage_s.at[j % NSLOT], wo_v.at[j], ssems.at[j % NSLOT])

    def smem_step(k):
        if isinstance(k, int):
            if k - 1 < NS:
                h2s(k - 1).wait()
                s2v(k - 1).start()
            if k + 1 < NS:
                if k + 1 - NSLOT >= 0:
                    s2v(k + 1 - NSLOT).wait()
                h2s(k + 1).start()
        else:
            raise NotImplementedError

    c_x = cp(x_hbm, x_v)
    c_wr = cp(wr_hbm, wr_v)
    c_wq = cp(wq_hbm, wq_v)
    c_wuk = cp(wuk_hbm, wuk_v)
    c_ckv = [cp(ckv_hbm.at[b], ckv_v.at[b]) for b in range(B)]
    c_wuv = cp(wuv_hbm, wuv_v)
    c_wg = cp(wg_hbm, wg_v)
    c_wu = cp(wu_hbm, wu_v)
    c_wd = []
    f0 = 0
    for n in WD_CHUNKS:
        c_wd.append(cp(wd_hbm.at[:, pl.ds(f0 * FC, n * FC)], wd_v.at[:, pl.ds(f0 * FC, n * FC)]))
        f0 += n
    c_wor = cp(wo_hbm.at[pl.ds(NS, H - NS), pl.ds(MS, M - MS)], wo_v.at[pl.ds(NS, H - NS), pl.ds(MS, M - MS)])
    c_wo = []
    h0 = NS
    for n in WO_CHUNKS:
        c_wo.append(cp(wo_hbm.at[pl.ds(h0, n), pl.ds(0, MS)], wo_v.at[pl.ds(h0, n), pl.ds(0, MS)]))
        h0 += n
    c_out = cp(o_v, o_hbm)
    c_wq.start()
    c_x.start()
    c_wr.start()
    for j in range(min(2, NS)):
        h2s(j).start()
    for c in [c_wuk] + c_ckv + [c_wuv, c_wg, c_wu] + c_wd + [c_wor] + c_wo:
        c.start()

    def rep_body(t, carry):
        row = lax.broadcasted_iota(jnp.int32, (128, 256), 0)
        col = lax.broadcasted_iota(jnp.int32, (128, 256), 1) + t * 256
        rep_v[t] = jnp.where((col >> 4) == row, 1.0, 0.0).astype(bf16)
        return carry
    lax.fori_loop(0, 8, rep_body, 0)

    def head_mask(width):
        row = lax.broadcasted_iota(jnp.int32, (B * HH, width), 0)
        col = lax.broadcasted_iota(jnp.int32, (B * HH, width), 1)
        return (row & (HH - 1)) == (col & (HH - 1))

    smem_step(1)
    c_x.wait()
    c_wr.wait()
    x = x_v[...].astype(f32)
    mu = jnp.mean(x, axis=-1, keepdims=True)
    xc = x - mu
    var = jnp.mean(xc * xc, axis=-1, keepdims=True)
    xn_b = (xc / jnp.sqrt(var + 1e-5)).astype(bf16)
    xn = xn_b.astype(f32)
    wr = wr_v[...].astype(f32).reshape(1, M)
    r = jnp.sum(xn * wr, axis=-1, keepdims=True)
    r_sel = jax.nn.sigmoid(r)

    mask256 = head_mask(256)
    for j in range(5):
        w = 128 if j < 4 else 64
        xj = xn_b[:, 128 * j:128 * j + w]
        for t in range(w // 16):
            xr = _dot(xj, rep_v[t, 0:w, :], NN)
            xb = jnp.concatenate(
                [jnp.broadcast_to(xr[b:b + 1, :], (HH, 256)) for b in range(B)], axis=0)
            xexp_v[8 * j + t] = jnp.where(mask256, xb, 0.0).astype(bf16)

    c_wq.wait()

    def q_body(t, carry):
        q0, q1 = carry
        l = xexp_v[t]
        m0 = pl.multiple_of(t * 16, 16)
        w0 = wq_v[pl.ds(m0, 16), 0:HH, :].reshape(256, D)
        w1 = wq_v[pl.ds(m0, 16), HH:H, :].reshape(256, D)
        return q0 + _dot(l, w0, NN), q1 + _dot(l, w1, NN)
    zq = jnp.zeros((B * HH, D), f32)
    q0, q1 = lax.fori_loop(0, 36, q_body, (zq, zq), unroll=4)
    scale = D ** -0.5
    qs = [(q0 * scale).astype(bf16), (q1 * scale).astype(bf16)]

    smem_step(2)
    c_wuk.wait()

    def qa_body(j, carry):
        for half in range(2):
            acc = jnp.zeros((B * HH, 128), f32)
            for t in range(8):
                c0 = pl.multiple_of(j * 128 + t * 16, 16)
                w = wuk_v[pl.ds(c0, 16), half * HH:(half + 1) * HH, :].reshape(256, D)
                rr = _dot(qs[half], w, NT)
                rm = jnp.where(mask256, rr, 0.0).astype(bf16)
                acc = acc + _dot(rm, rep_v[t], NT)
            accb = acc.astype(bf16)
            for b in range(B):
                qabs_v[j, b, half * HH:(half + 1) * HH, :] = accb[b * HH:(b + 1) * HH, :]
        return carry
    lax.fori_loop(0, 4, qa_body, 0)

    def attn(b):
        qa = jnp.concatenate([qabs_v[j, b] for j in range(4)], axis=1)

        def s_body(i, mx):
            k0 = pl.multiple_of(i * KC, KC)
            s = _dot(qa, ckv_v[b, pl.ds(k0, KC), :], NT)
            s_v[i] = s
            m = s[:, 0:128]
            for u in range(1, KC // 128):
                m = jnp.maximum(m, s[:, u * 128:(u + 1) * 128])
            return jnp.maximum(mx, m)
        mx = lax.fori_loop(0, SK // KC, s_body, jnp.full((H, 128), -jnp.inf, f32))
        mrow = jnp.max(mx, axis=-1, keepdims=True)

        def pv_body(i, carry2):
            acc, ls = carry2
            k0 = pl.multiple_of(i * KC, KC)
            p = jnp.exp(s_v[i] - mrow)
            for u in range(KC // 128):
                ls = ls + p[:, u * 128:(u + 1) * 128]
            acc = acc + _dot(p.astype(bf16), ckv_v[b, pl.ds(k0, KC), :], NN)
            return acc, ls
        acc, ls = lax.fori_loop(0, SK // KC, pv_body,
                                (jnp.zeros((H, DC), f32), jnp.zeros((H, 128), f32)))
        l = jnp.sum(ls, axis=-1, keepdims=True)
        cc = (acc / l).astype(bf16)
        for j in range(4):
            ctxc_v[j, b] = cc[:, j * 128:(j + 1) * 128]

    for b in range(B):
        smem_step(3 + b)
        c_ckv[b].wait()
        attn(b)

    smem_step(7)
    c_wuv.wait()

    def v_body(j, carry):
        out = []
        for half in range(2):
            acc = carry[half]
            l = jnp.concatenate(
                [ctxc_v[j, b, half * HH:(half + 1) * HH, :] for b in range(B)], axis=0)
            for t in range(8):
                c0 = pl.multiple_of(j * 128 + t * 16, 16)
                lr = _dot(l, rep_v[t], NN)
                le = jnp.where(mask256, lr, 0.0).astype(bf16)
                w = wuv_v[pl.ds(c0, 16), half * HH:(half + 1) * HH, :].reshape(256, D)
                acc = acc + _dot(le, w, NN)
            out.append(acc)
        return tuple(out)
    ctx0, ctx1 = lax.fori_loop(0, 4, v_body, (zq, zq))
    prow = lax.broadcasted_iota(jnp.int32, (8 * HH, B * HH), 0)
    pcol = lax.broadcasted_iota(jnp.int32, (8 * HH, B * HH), 1)
    perm = jnp.where(((prow >> 3) == (pcol & (HH - 1))) & ((prow & 7) == (pcol >> 4)), 1.0, 0.0).astype(bf16)
    for half, cx in enumerate((ctx0, ctx1)):
        cp_ = _dot(perm, cx.astype(bf16), NN)
        for hh in range(HH):
            ctxo_v[half * HH + hh] = cp_[8 * hh:8 * hh + 8, :]

    smem_step(8)
    c_wg.wait()

    def g_body(i, carry):
        f0 = pl.multiple_of(i * FC, FC)
        g = _dot(xn_b, wg_v[:, pl.ds(f0, FC)], NN)
        h_v[i] = g * jax.nn.sigmoid(g)
        return carry
    lax.fori_loop(0, F // FC, g_body, 0)
    smem_step(9)
    c_wu.wait()

    def u_body(i, carry):
        f0 = pl.multiple_of(i * FC, FC)
        h_v[i] = h_v[i] * _dot(xn_b, wu_v[:, pl.ds(f0, FC)], NN)
        return carry
    lax.fori_loop(0, F // FC, u_body, 0)
    smem_step(10)
    assert NS <= 10

    def o_chunk(hs, n, m0, m1, tag='o'):
        if tag in skip:
            return jnp.zeros((8, m1 - m0), f32)
        l = jnp.concatenate([ctxo_v[hs + i] for i in range(n)], axis=1).astype(bf16)
        w = jnp.concatenate([wo_v[hs + i, m0:m1, :] for i in range(n)], axis=1)
        return _dot(l, w, NT)

    def d_body(i, y):
        f0 = pl.multiple_of(i * FC, FC)
        return y + _dot(h_v[i].astype(bf16), wd_v[:, pl.ds(f0, FC)], NT)
    y = jnp.zeros((B, M), f32)
    s = jnp.zeros((8, M), f32)
    f0 = 0
    for idx, (n, c) in enumerate(zip(WD_CHUNKS, c_wd)):
        if idx == len(WD_CHUNKS) - 1 and NS > 0:
            for j in range(max(0, NS - NSLOT), NS):
                s2v(j).wait()
            s = o_chunk(0, NS, 0, M, 'ostage')
        c.wait()
        if 'down' not in skip:
            y = lax.fori_loop(f0, f0 + n, d_body, y)
        f0 += n
    z = xn + y * r_sel
    gate = z * jax.nn.sigmoid(z)

    xg_v[...] = jnp.zeros(xg_v.shape, f32)
    xg_v[0, 0:B, :] = x
    xg_v[1, 0:B, :] = gate
    c_wor.wait()
    s_hi = s[:, MS:M] + o_chunk(NS, H - NS, MS, M, 'orem')
    o_v[:, MS:M] = (xg_v[0, :, MS:M] + s_hi * xg_v[1, :, MS:M])[0:B, :].astype(bf16)
    s = s[:, 0:MS]
    h0 = NS
    for idx, (n, c) in enumerate(zip(WO_CHUNKS, c_wo)):
        if idx == len(WO_CHUNKS) - 1:
            g_lo = xg_v[1, :, 0:MS]
            base = xg_v[0, :, 0:MS] + s * g_lo
            c.wait()
            o_v[:, 0:MS] = (base + o_chunk(h0, n, 0, MS, 'olast') * g_lo)[0:B, :].astype(bf16)
        else:
            c.wait()
            s = s + o_chunk(h0, n, 0, MS)
        h0 += n

    c_out.start()
    c_out.wait()


  @jax.jit
  def kernel_fn(A_x, A_c_kv, A_w_q, A_w_uk, A_w_uv, A_w_o, B_x, B_w_r, B_w_gate, B_w_up, B_w_down):
    x = A_x.reshape(B, M)
    wo_t = jnp.transpose(A_w_o, (0, 2, 1))
    wd_t = B_w_down.T
    any_spec = pl.BlockSpec(memory_space=pl.ANY)
    nsem = 4 + B + 3 + len(WD_CHUNKS) + len(WO_CHUNKS) + 2
    out = pl.pallas_call(
        _kernel,
        out_shape=jax.ShapeDtypeStruct((B, M), bf16),
        in_specs=[any_spec] * 10,
        out_specs=any_spec,
        scratch_shapes=[
            pltpu.VMEM((B, M), bf16),
            pltpu.VMEM((M,), bf16),
            pltpu.VMEM((B, SK, DC), bf16),
            pltpu.VMEM((M, H, D), bf16),
            pltpu.VMEM((DC, H, D), bf16),
            pltpu.VMEM((DC, H, D), bf16),
            pltpu.VMEM((H, M, D), bf16),
            pltpu.VMEM((M, F), bf16),
            pltpu.VMEM((M, F), bf16),
            pltpu.VMEM((M, F), bf16),
            pltpu.VMEM((B, M), bf16),
            pltpu.VMEM((8, 128, 256), bf16),
            pltpu.VMEM((36, B * HH, 256), bf16),
            pltpu.VMEM((4, B, H, 128), bf16),
            pltpu.VMEM((SK // KC, H, KC), f32),
            pltpu.VMEM((H, 8, D), f32),
            pltpu.VMEM((4, B, H, 128), bf16),
            pltpu.VMEM((2, 8, M), f32),
            pltpu.VMEM((F // FC, B, FC), f32),
            pltpu.SMEM((NSLOT, M, D), bf16),
            pltpu.SemaphoreType.DMA((nsem,)),
            pltpu.SemaphoreType.DMA((NSLOT,)),
            pltpu.SemaphoreType.DMA((NSLOT,)),
        ],
        compiler_params=pltpu.CompilerParams(
            vmem_limit_bytes=100 * 1024 * 1024,
            disable_semaphore_checks=dsc,
            disable_bounds_checks=dbc,
        ),
    )(x, B_w_r, A_c_kv, A_w_q, A_w_uk, A_w_uv, wo_t, B_w_gate, B_w_up, wd_t)
    return out.reshape(B, 1, M)
  return kernel_fn

pallas_recurrent_scan__compressed_kv_cla__moe_arch_mod__decode_kernel = make()
```

```python
import jax
import jax.numpy as jnp
from jax import lax
import jax.experimental.pallas as pl
import jax.experimental.pallas.tpu as pltpu

B, H, SK, D, M = 4, 32, 4096, 128, 576
DC = 4 * D
F = 4608
HH = 16
KC = 512
FC = 512
MS = 512
NS = 10
NSLOT = 4
WO_CHUNKS = (8, 6, 4, 2, 1, 1)
WD_CHUNKS = (3, 3, 3)
EPS = 1e-5

f32 = jnp.float32
bf16 = jnp.bfloat16
NN = (((1,), (0,)), ((), ()))
NT = (((1,), (1,)), ((), ()))

assert NS + sum(WO_CHUNKS) == H and sum(WD_CHUNKS) * FC == F and NSLOT <= NS <= 10


def _dot(a, b, dims):
    return lax.dot_general(a, b, dims, preferred_element_type=f32)


def _kernel(x_hbm, wr_hbm, ckv_hbm, wq_hbm, wuk_hbm, wuv_hbm, wo_hbm, wg_hbm, wu_hbm, wd_hbm,
            o_hbm,
            x_v, wr_v, ckv_v, wq_v, wuk_v, wuv_v, wo_v, wg_v, wu_v, wd_v, o_v,
            rep_v, xexp_v, qabs_v, s_v, ctxc_v, ctxo_v, xg_v, h_v, stage_s,
            sems, hsems, ssems):
    n_sems = [0]

    def copy(src, dst):
        c = pltpu.make_async_copy(src, dst, sems.at[n_sems[0]])
        n_sems[0] += 1
        return c

    def h2s(j):
        return pltpu.make_async_copy(wo_hbm.at[j], stage_s.at[j % NSLOT], hsems.at[j % NSLOT])

    def s2v(j):
        return pltpu.make_async_copy(stage_s.at[j % NSLOT], wo_v.at[j], ssems.at[j % NSLOT])

    def smem_step(k):
        if k - 1 < NS:
            h2s(k - 1).wait()
            s2v(k - 1).start()
        if k + 1 < NS:
            if k + 1 >= NSLOT:
                s2v(k + 1 - NSLOT).wait()
            h2s(k + 1).start()

    c_wq = copy(wq_hbm, wq_v)
    c_x = copy(x_hbm, x_v)
    c_wr = copy(wr_hbm, wr_v)
    c_wuk = copy(wuk_hbm, wuk_v)
    c_ckv = [copy(ckv_hbm.at[b], ckv_v.at[b]) for b in range(B)]
    c_wuv = copy(wuv_hbm, wuv_v)
    c_wg = copy(wg_hbm, wg_v)
    c_wu = copy(wu_hbm, wu_v)
    c_wd = []
    f0 = 0
    for n in WD_CHUNKS:
        cols = pl.ds(f0 * FC, n * FC)
        c_wd.append(copy(wd_hbm.at[:, cols], wd_v.at[:, cols]))
        f0 += n
    c_wo_hi = copy(wo_hbm.at[pl.ds(NS, H - NS), pl.ds(MS, M - MS)],
                   wo_v.at[pl.ds(NS, H - NS), pl.ds(MS, M - MS)])
    c_wo = []
    h0 = NS
    for n in WO_CHUNKS:
        c_wo.append(copy(wo_hbm.at[pl.ds(h0, n), pl.ds(0, MS)], wo_v.at[pl.ds(h0, n), pl.ds(0, MS)]))
        h0 += n
    c_out = copy(o_v, o_hbm)

    c_wq.start()
    c_x.start()
    c_wr.start()
    h2s(0).start()
    h2s(1).start()
    for c in [c_wuk] + c_ckv + [c_wuv, c_wg, c_wu] + c_wd + [c_wo_hi] + c_wo:
        c.start()

    def rep_body(t, carry):
        row = lax.broadcasted_iota(jnp.int32, (128, 256), 0)
        col = lax.broadcasted_iota(jnp.int32, (128, 256), 1) + t * 256
        rep_v[t] = jnp.where((col >> 4) == row, 1.0, 0.0).astype(bf16)
        return carry
    lax.fori_loop(0, 8, rep_body, 0)

    head_mask = ((lax.broadcasted_iota(jnp.int32, (B * HH, 256), 0) & (HH - 1))
                 == (lax.broadcasted_iota(jnp.int32, (B * HH, 256), 1) & (HH - 1)))

    smem_step(1)
    c_x.wait()
    c_wr.wait()
    x = x_v[...].astype(f32)
    xc = x - jnp.mean(x, axis=-1, keepdims=True)
    var = jnp.mean(xc * xc, axis=-1, keepdims=True)
    xn_b = (xc / jnp.sqrt(var + EPS)).astype(bf16)
    xn = xn_b.astype(f32)
    r = jnp.sum(xn * wr_v[...].astype(f32).reshape(1, M), axis=-1, keepdims=True)
    r_sel = jax.nn.sigmoid(r)

    for j in range(5):
        w = 128 if j < 4 else M - 512
        xj = xn_b[:, 128 * j:128 * j + w]
        for t in range(w // 16):
            xr = _dot(xj, rep_v[t, 0:w, :], NN)
            xb = jnp.concatenate(
                [jnp.broadcast_to(xr[b:b + 1, :], (HH, 256)) for b in range(B)], axis=0)
            xexp_v[8 * j + t] = jnp.where(head_mask, xb, 0.0).astype(bf16)

    c_wq.wait()

    def q_body(t, carry):
        q0, q1 = carry
        lhs = xexp_v[t]
        m0 = pl.multiple_of(t * 16, 16)
        w0 = wq_v[pl.ds(m0, 16), 0:HH, :].reshape(256, D)
        w1 = wq_v[pl.ds(m0, 16), HH:H, :].reshape(256, D)
        return q0 + _dot(lhs, w0, NN), q1 + _dot(lhs, w1, NN)
    zero_q = jnp.zeros((B * HH, D), f32)
    q0, q1 = lax.fori_loop(0, M // 16, q_body, (zero_q, zero_q), unroll=4)
    scale = D ** -0.5
    qs = [(q0 * scale).astype(bf16), (q1 * scale).astype(bf16)]

    smem_step(2)
    c_wuk.wait()

    def qa_body(j, carry):
        for half in range(2):
            acc = jnp.zeros((B * HH, 128), f32)
            for t in range(8):
                c0 = pl.multiple_of(j * 128 + t * 16, 16)
                w = wuk_v[pl.ds(c0, 16), half * HH:(half + 1) * HH, :].reshape(256, D)
                allpairs = _dot(qs[half], w, NT)
                own = jnp.where(head_mask, allpairs, 0.0).astype(bf16)
                acc = acc + _dot(own, rep_v[t], NT)
            acc = acc.astype(bf16)
            for b in range(B):
                qabs_v[j, b, half * HH:(half + 1) * HH, :] = acc[b * HH:(b + 1) * HH, :]
        return carry
    lax.fori_loop(0, DC // 128, qa_body, 0)

    def attend(b):
        qa = jnp.concatenate([qabs_v[j, b] for j in range(DC // 128)], axis=1)

        def score_body(i, mx):
            k0 = pl.multiple_of(i * KC, KC)
            s = _dot(qa, ckv_v[b, pl.ds(k0, KC), :], NT)
            s_v[i] = s
            for u in range(KC // 128):
                mx = jnp.maximum(mx, s[:, u * 128:(u + 1) * 128])
            return mx
        mx = lax.fori_loop(0, SK // KC, score_body, jnp.full((H, 128), -jnp.inf, f32))
        row_max = jnp.max(mx, axis=-1, keepdims=True)

        def pv_body(i, carry):
            acc, den = carry
            k0 = pl.multiple_of(i * KC, KC)
            p = jnp.exp(s_v[i] - row_max)
            for u in range(KC // 128):
                den = den + p[:, u * 128:(u + 1) * 128]
            return acc + _dot(p.astype(bf16), ckv_v[b, pl.ds(k0, KC), :], NN), den
        acc, den = lax.fori_loop(0, SK // KC, pv_body,
                                 (jnp.zeros((H, DC), f32), jnp.zeros((H, 128), f32)))
        cc = (acc / jnp.sum(den, axis=-1, keepdims=True)).astype(bf16)
        for j in range(DC // 128):
            ctxc_v[j, b] = cc[:, j * 128:(j + 1) * 128]

    for b in range(B):
        smem_step(3 + b)
        c_ckv[b].wait()
        attend(b)

    smem_step(7)
    c_wuv.wait()

    def v_body(j, carry):
        out = []
        for half in range(2):
            acc = carry[half]
            lhs = jnp.concatenate(
                [ctxc_v[j, b, half * HH:(half + 1) * HH, :] for b in range(B)], axis=0)
            for t in range(8):
                c0 = pl.multiple_of(j * 128 + t * 16, 16)
                rep = _dot(lhs, rep_v[t], NN)
                own = jnp.where(head_mask, rep, 0.0).astype(bf16)
                w = wuv_v[pl.ds(c0, 16), half * HH:(half + 1) * HH, :].reshape(256, D)
                acc = acc + _dot(own, w, NN)
            out.append(acc)
        return tuple(out)
    ctx_halves = lax.fori_loop(0, DC // 128, v_body, (zero_q, zero_q))

    prow = lax.broadcasted_iota(jnp.int32, (8 * HH, B * HH), 0)
    pcol = lax.broadcasted_iota(jnp.int32, (8 * HH, B * HH), 1)
    perm = jnp.where(((prow >> 3) == (pcol & (HH - 1))) & ((prow & 7) == (pcol >> 4)),
                     1.0, 0.0).astype(bf16)
    for half, ctx in enumerate(ctx_halves):
        slabs = _dot(perm, ctx.astype(bf16), NN)
        for hh in range(HH):
            ctxo_v[half * HH + hh] = slabs[8 * hh:8 * hh + 8, :]

    smem_step(8)
    c_wg.wait()

    def gate_body(i, carry):
        c0 = pl.multiple_of(i * FC, FC)
        g = _dot(xn_b, wg_v[:, pl.ds(c0, FC)], NN)
        h_v[i] = g * jax.nn.sigmoid(g)
        return carry
    lax.fori_loop(0, F // FC, gate_body, 0)

    smem_step(9)
    c_wu.wait()

    def up_body(i, carry):
        c0 = pl.multiple_of(i * FC, FC)
        h_v[i] = h_v[i] * _dot(xn_b, wu_v[:, pl.ds(c0, FC)], NN)
        return carry
    lax.fori_loop(0, F // FC, up_body, 0)
    smem_step(10)

    def out_proj(hs, n, m0, m1):
        lhs = jnp.concatenate([ctxo_v[hs + i] for i in range(n)], axis=1).astype(bf16)
        w = jnp.concatenate([wo_v[hs + i, m0:m1, :] for i in range(n)], axis=1)
        return _dot(lhs, w, NT)

    def down_body(i, y):
        c0 = pl.multiple_of(i * FC, FC)
        return y + _dot(h_v[i].astype(bf16), wd_v[:, pl.ds(c0, FC)], NT)

    y = jnp.zeros((B, M), f32)
    f0 = 0
    for idx, (n, c) in enumerate(zip(WD_CHUNKS, c_wd)):
        if idx == len(WD_CHUNKS) - 1:
            for j in range(NS - NSLOT, NS):
                s2v(j).wait()
            s = out_proj(0, NS, 0, M)
        c.wait()
        y = lax.fori_loop(f0, f0 + n, down_body, y)
        f0 += n
    z = xn + y * r_sel
    gate = z * jax.nn.sigmoid(z)

    xg_v[...] = jnp.zeros(xg_v.shape, f32)
    xg_v[0, 0:B, :] = x
    xg_v[1, 0:B, :] = gate

    c_wo_hi.wait()
    s_hi = s[:, MS:M] + out_proj(NS, H - NS, MS, M)
    o_v[:, MS:M] = (xg_v[0, :, MS:M] + s_hi * xg_v[1, :, MS:M])[0:B, :].astype(bf16)

    s = s[:, 0:MS]
    h0 = NS
    for n, c in zip(WO_CHUNKS[:-1], c_wo[:-1]):
        c.wait()
        s = s + out_proj(h0, n, 0, MS)
        h0 += n
    gate_lo = xg_v[1, :, 0:MS]
    base = xg_v[0, :, 0:MS] + s * gate_lo
    c_wo[-1].wait()
    o_v[:, 0:MS] = (base + out_proj(h0, WO_CHUNKS[-1], 0, MS) * gate_lo)[0:B, :].astype(bf16)

    c_out.start()
    c_out.wait()


@jax.jit
def pallas_recurrent_scan__compressed_kv_cla__moe_arch_mod__decode_kernel(
    A_x: jax.Array,
    A_c_kv: jax.Array,
    A_w_q: jax.Array,
    A_w_uk: jax.Array,
    A_w_uv: jax.Array,
    A_w_o: jax.Array,
    B_x: jax.Array,
    B_w_r: jax.Array,
    B_w_gate: jax.Array,
    B_w_up: jax.Array,
    B_w_down: jax.Array,
):
    del B_x
    x = A_x.reshape(B, M)
    wo_t = jnp.transpose(A_w_o, (0, 2, 1))
    wd_t = B_w_down.T
    hbm = pl.BlockSpec(memory_space=pl.ANY)
    n_sems = 4 + B + 3 + len(WD_CHUNKS) + 1 + len(WO_CHUNKS) + 1
    out = pl.pallas_call(
        _kernel,
        out_shape=jax.ShapeDtypeStruct((B, M), bf16),
        in_specs=[hbm] * 10,
        out_specs=hbm,
        scratch_shapes=[
            pltpu.VMEM((B, M), bf16),
            pltpu.VMEM((M,), bf16),
            pltpu.VMEM((B, SK, DC), bf16),
            pltpu.VMEM((M, H, D), bf16),
            pltpu.VMEM((DC, H, D), bf16),
            pltpu.VMEM((DC, H, D), bf16),
            pltpu.VMEM((H, M, D), bf16),
            pltpu.VMEM((M, F), bf16),
            pltpu.VMEM((M, F), bf16),
            pltpu.VMEM((M, F), bf16),
            pltpu.VMEM((B, M), bf16),
            pltpu.VMEM((8, 128, 256), bf16),
            pltpu.VMEM((M // 16, B * HH, 256), bf16),
            pltpu.VMEM((DC // 128, B, H, 128), bf16),
            pltpu.VMEM((SK // KC, H, KC), f32),
            pltpu.VMEM((DC // 128, B, H, 128), bf16),
            pltpu.VMEM((H, 8, D), f32),
            pltpu.VMEM((2, 8, M), f32),
            pltpu.VMEM((F // FC, B, FC), f32),
            pltpu.SMEM((NSLOT, M, D), bf16),
            pltpu.SemaphoreType.DMA((n_sems,)),
            pltpu.SemaphoreType.DMA((NSLOT,)),
            pltpu.SemaphoreType.DMA((NSLOT,)),
        ],
        compiler_params=pltpu.CompilerParams(
            vmem_limit_bytes=72 * 1024 * 1024,
            disable_semaphore_checks=True,
        ),
    )(x, B_w_r, A_c_kv, A_w_q, A_w_uk, A_w_uv, wo_t, B_w_gate, B_w_up, wd_t)
    return out.reshape(B, 1, M)
```

```python
import jax
import jax.numpy as jnp
from jax import lax
import jax.experimental.pallas as pl
import jax.experimental.pallas.tpu as pltpu

B, H, SK, D, M = 4, 32, 4096, 128, 576
DC = 4 * D
F = 4608
HH = 16
KC = 512
FC = 512
MS = 512
NS = 10
NSLOT = 4
WO_CHUNKS = (8, 6, 4, 2, 1, 1)
WD_CHUNKS = (3, 3, 3)
EPS = 1e-5

f32 = jnp.float32
bf16 = jnp.bfloat16
NN = (((1,), (0,)), ((), ()))
NT = (((1,), (1,)), ((), ()))

assert NS + sum(WO_CHUNKS) == H and sum(WD_CHUNKS) * FC == F and NSLOT <= NS <= 10


def _dot(a, b, dims):
    return lax.dot_general(a, b, dims, preferred_element_type=f32)


def _r(v):
    return v.astype(bf16).astype(f32)


def _kernel(x_hbm, wr_hbm, ckv_hbm, wq_hbm, wuk_hbm, wuv_hbm, wo_hbm, wg_hbm, wu_hbm, wd_hbm,
            o_hbm,
            x_v, wr_v, ckv_v, wq_v, wuk_v, wuv_v, wo_v, wg_v, wu_v, wd_v, o_v,
            rep_v, xexp_v, qabs_v, s_v, ctxc_v, ctxo_v, xg_v, h_v, stage_s,
            sems, hsems, ssems):
    n_sems = [0]

    def copy(src, dst):
        c = pltpu.make_async_copy(src, dst, sems.at[n_sems[0]])
        n_sems[0] += 1
        return c

    def h2s(j):
        return pltpu.make_async_copy(wo_hbm.at[j], stage_s.at[j % NSLOT], hsems.at[j % NSLOT])

    def s2v(j):
        return pltpu.make_async_copy(stage_s.at[j % NSLOT], wo_v.at[j], ssems.at[j % NSLOT])

    def smem_step(k):
        if k - 1 < NS:
            h2s(k - 1).wait()
            s2v(k - 1).start()
        if k + 1 < NS:
            if k + 1 >= NSLOT:
                s2v(k + 1 - NSLOT).wait()
            h2s(k + 1).start()

    c_wq = copy(wq_hbm, wq_v)
    c_x = copy(x_hbm, x_v)
    c_wr = copy(wr_hbm, wr_v)
    c_wuk = copy(wuk_hbm, wuk_v)
    c_ckv = [copy(ckv_hbm.at[b], ckv_v.at[b]) for b in range(B)]
    c_wuv = copy(wuv_hbm, wuv_v)
    c_wg = copy(wg_hbm, wg_v)
    c_wu = copy(wu_hbm, wu_v)
    c_wd = []
    f0 = 0
    for n in WD_CHUNKS:
        cols = pl.ds(f0 * FC, n * FC)
        c_wd.append(copy(wd_hbm.at[:, cols], wd_v.at[:, cols]))
        f0 += n
    c_wo_hi = copy(wo_hbm.at[pl.ds(NS, H - NS), pl.ds(MS, M - MS)],
                   wo_v.at[pl.ds(NS, H - NS), pl.ds(MS, M - MS)])
    c_wo = []
    h0 = NS
    for n in WO_CHUNKS:
        c_wo.append(copy(wo_hbm.at[pl.ds(h0, n), pl.ds(0, MS)], wo_v.at[pl.ds(h0, n), pl.ds(0, MS)]))
        h0 += n
    c_out = copy(o_v, o_hbm)

    c_wq.start()
    c_x.start()
    c_wr.start()
    h2s(0).start()
    h2s(1).start()
    for c in [c_wuk] + c_ckv + [c_wuv, c_wg, c_wu] + c_wd + [c_wo_hi] + c_wo:
        c.start()

    def rep_body(t, carry):
        row = lax.broadcasted_iota(jnp.int32, (128, 256), 0)
        col = lax.broadcasted_iota(jnp.int32, (128, 256), 1) + t * 256
        rep_v[t] = jnp.where((col >> 4) == row, 1.0, 0.0).astype(bf16)
        return carry
    lax.fori_loop(0, 8, rep_body, 0)

    head_mask = ((lax.broadcasted_iota(jnp.int32, (B * HH, 256), 0) & (HH - 1))
                 == (lax.broadcasted_iota(jnp.int32, (B * HH, 256), 1) & (HH - 1)))

    smem_step(1)
    c_x.wait()
    c_wr.wait()
    x = x_v[...].astype(f32)
    mean = jnp.mean(x, axis=-1, keepdims=True)
    var = jnp.mean((x - mean) * (x - mean), axis=-1, keepdims=True)
    std = _r(jnp.sqrt(_r(_r(var) + EPS)))
    xn_b = (_r(x - _r(mean)) / std).astype(bf16)
    xn = xn_b.astype(f32)
    r = jnp.sum(xn * wr_v[...].astype(f32).reshape(1, M), axis=-1, keepdims=True)
    r_sel = _r(jax.nn.sigmoid(_r(r)))

    for j in range(5):
        w = 128 if j < 4 else M - 512
        xj = xn_b[:, 128 * j:128 * j + w]
        for t in range(w // 16):
            xr = _dot(xj, rep_v[t, 0:w, :], NN)
            xb = jnp.concatenate(
                [jnp.broadcast_to(xr[b:b + 1, :], (HH, 256)) for b in range(B)], axis=0)
            xexp_v[8 * j + t] = jnp.where(head_mask, xb, 0.0).astype(bf16)

    c_wq.wait()

    def q_body(t, carry):
        q0, q1 = carry
        lhs = xexp_v[t]
        m0 = pl.multiple_of(t * 16, 16)
        w0 = wq_v[pl.ds(m0, 16), 0:HH, :].reshape(256, D)
        w1 = wq_v[pl.ds(m0, 16), HH:H, :].reshape(256, D)
        return q0 + _dot(lhs, w0, NN), q1 + _dot(lhs, w1, NN)
    zero_q = jnp.zeros((B * HH, D), f32)
    q0, q1 = lax.fori_loop(0, M // 16, q_body, (zero_q, zero_q), unroll=4)
    scale = D ** -0.5
    qs = [(q0 * scale).astype(bf16), (q1 * scale).astype(bf16)]

    smem_step(2)
    c_wuk.wait()

    def qa_body(j, carry):
        for half in range(2):
            acc = jnp.zeros((B * HH, 128), f32)
            for t in range(8):
                c0 = pl.multiple_of(j * 128 + t * 16, 16)
                w = wuk_v[pl.ds(c0, 16), half * HH:(half + 1) * HH, :].reshape(256, D)
                allpairs = _dot(qs[half], w, NT)
                own = jnp.where(head_mask, allpairs, 0.0).astype(bf16)
                acc = acc + _dot(own, rep_v[t], NT)
            acc = acc.astype(bf16)
            for b in range(B):
                qabs_v[j, b, half * HH:(half + 1) * HH, :] = acc[b * HH:(b + 1) * HH, :]
        return carry
    lax.fori_loop(0, DC // 128, qa_body, 0)

    def attend(b):
        qa = jnp.concatenate([qabs_v[j, b] for j in range(DC // 128)], axis=1)

        def score_body(i, mx):
            k0 = pl.multiple_of(i * KC, KC)
            s = _dot(qa, ckv_v[b, pl.ds(k0, KC), :], NT)
            s_v[i] = s
            for u in range(KC // 128):
                mx = jnp.maximum(mx, s[:, u * 128:(u + 1) * 128])
            return mx
        mx = lax.fori_loop(0, SK // KC, score_body, jnp.full((H, 128), -jnp.inf, f32))
        row_max = jnp.max(mx, axis=-1, keepdims=True)

        def pv_body(i, carry):
            acc, den = carry
            k0 = pl.multiple_of(i * KC, KC)
            p = jnp.exp(s_v[i] - row_max)
            for u in range(KC // 128):
                den = den + p[:, u * 128:(u + 1) * 128]
            return acc + _dot(p.astype(bf16), ckv_v[b, pl.ds(k0, KC), :], NN), den
        acc, den = lax.fori_loop(0, SK // KC, pv_body,
                                 (jnp.zeros((H, DC), f32), jnp.zeros((H, 128), f32)))
        cc = (acc / jnp.sum(den, axis=-1, keepdims=True)).astype(bf16)
        for j in range(DC // 128):
            ctxc_v[j, b] = cc[:, j * 128:(j + 1) * 128]

    for b in range(B):
        smem_step(3 + b)
        c_ckv[b].wait()
        attend(b)

    smem_step(7)
    c_wuv.wait()

    def v_body(j, carry):
        out = []
        for half in range(2):
            acc = carry[half]
            lhs = jnp.concatenate(
                [ctxc_v[j, b, half * HH:(half + 1) * HH, :] for b in range(B)], axis=0)
            for t in range(8):
                c0 = pl.multiple_of(j * 128 + t * 16, 16)
                rep = _dot(lhs, rep_v[t], NN)
                own = jnp.where(head_mask, rep, 0.0).astype(bf16)
                w = wuv_v[pl.ds(c0, 16), half * HH:(half + 1) * HH, :].reshape(256, D)
                acc = acc + _dot(own, w, NN)
            out.append(acc)
        return tuple(out)
    ctx_halves = lax.fori_loop(0, DC // 128, v_body, (zero_q, zero_q))

    prow = lax.broadcasted_iota(jnp.int32, (8 * HH, B * HH), 0)
    pcol = lax.broadcasted_iota(jnp.int32, (8 * HH, B * HH), 1)
    perm = jnp.where(((prow >> 3) == (pcol & (HH - 1))) & ((prow & 7) == (pcol >> 4)),
                     1.0, 0.0).astype(bf16)
    for half, ctx in enumerate(ctx_halves):
        slabs = _dot(perm, ctx.astype(bf16), NN)
        for hh in range(HH):
            ctxo_v[half * HH + hh] = slabs[8 * hh:8 * hh + 8, :]

    smem_step(8)
    c_wg.wait()

    def gate_body(i, carry):
        c0 = pl.multiple_of(i * FC, FC)
        g = _r(_dot(xn_b, wg_v[:, pl.ds(c0, FC)], NN))
        h_v[i] = _r(g * jax.nn.sigmoid(g))
        return carry
    lax.fori_loop(0, F // FC, gate_body, 0)

    smem_step(9)
    c_wu.wait()

    def up_body(i, carry):
        c0 = pl.multiple_of(i * FC, FC)
        h_v[i] = h_v[i] * _r(_dot(xn_b, wu_v[:, pl.ds(c0, FC)], NN))
        return carry
    lax.fori_loop(0, F // FC, up_body, 0)
    smem_step(10)

    def out_proj(hs, n, m0, m1):
        lhs = jnp.concatenate([ctxo_v[hs + i] for i in range(n)], axis=1).astype(bf16)
        w = jnp.concatenate([wo_v[hs + i, m0:m1, :] for i in range(n)], axis=1)
        return _dot(lhs, w, NT)

    def down_body(i, y):
        c0 = pl.multiple_of(i * FC, FC)
        return y + _dot(h_v[i].astype(bf16), wd_v[:, pl.ds(c0, FC)], NT)

    y = jnp.zeros((B, M), f32)
    f0 = 0
    for idx, (n, c) in enumerate(zip(WD_CHUNKS, c_wd)):
        if idx == len(WD_CHUNKS) - 1:
            for j in range(NS - NSLOT, NS):
                s2v(j).wait()
            s = out_proj(0, NS, 0, M)
        c.wait()
        y = lax.fori_loop(f0, f0 + n, down_body, y)
        f0 += n
    z = _r(xn + _r(_r(y) * r_sel))
    gate = _r(z * jax.nn.sigmoid(z))

    xg_v[...] = jnp.zeros(xg_v.shape, f32)
    xg_v[0, 0:B, :] = x
    xg_v[1, 0:B, :] = gate

    c_wo_hi.wait()
    s_hi = s[:, MS:M] + out_proj(NS, H - NS, MS, M)
    o_v[:, MS:M] = (xg_v[0, :, MS:M] + s_hi * xg_v[1, :, MS:M])[0:B, :].astype(bf16)

    s = s[:, 0:MS]
    h0 = NS
    for n, c in zip(WO_CHUNKS[:-1], c_wo[:-1]):
        c.wait()
        s = s + out_proj(h0, n, 0, MS)
        h0 += n
    gate_lo = xg_v[1, :, 0:MS]
    base = xg_v[0, :, 0:MS] + s * gate_lo
    c_wo[-1].wait()
    o_v[:, 0:MS] = (base + out_proj(h0, WO_CHUNKS[-1], 0, MS) * gate_lo)[0:B, :].astype(bf16)

    c_out.start()
    c_out.wait()


@jax.jit
def pallas_recurrent_scan__compressed_kv_cla__moe_arch_mod__decode_kernel(
    A_x: jax.Array,
    A_c_kv: jax.Array,
    A_w_q: jax.Array,
    A_w_uk: jax.Array,
    A_w_uv: jax.Array,
    A_w_o: jax.Array,
    B_x: jax.Array,
    B_w_r: jax.Array,
    B_w_gate: jax.Array,
    B_w_up: jax.Array,
    B_w_down: jax.Array,
):
    del B_x
    x = A_x.reshape(B, M)
    wo_t = jnp.transpose(A_w_o, (0, 2, 1))
    wd_t = B_w_down.T
    hbm = pl.BlockSpec(memory_space=pl.ANY)
    n_sems = 4 + B + 3 + len(WD_CHUNKS) + 1 + len(WO_CHUNKS) + 1
    out = pl.pallas_call(
        _kernel,
        out_shape=jax.ShapeDtypeStruct((B, M), bf16),
        in_specs=[hbm] * 10,
        out_specs=hbm,
        scratch_shapes=[
            pltpu.VMEM((B, M), bf16),
            pltpu.VMEM((M,), bf16),
            pltpu.VMEM((B, SK, DC), bf16),
            pltpu.VMEM((M, H, D), bf16),
            pltpu.VMEM((DC, H, D), bf16),
            pltpu.VMEM((DC, H, D), bf16),
            pltpu.VMEM((H, M, D), bf16),
            pltpu.VMEM((M, F), bf16),
            pltpu.VMEM((M, F), bf16),
            pltpu.VMEM((M, F), bf16),
            pltpu.VMEM((B, M), bf16),
            pltpu.VMEM((8, 128, 256), bf16),
            pltpu.VMEM((M // 16, B * HH, 256), bf16),
            pltpu.VMEM((DC // 128, B, H, 128), bf16),
            pltpu.VMEM((SK // KC, H, KC), f32),
            pltpu.VMEM((DC // 128, B, H, 128), bf16),
            pltpu.VMEM((H, 8, D), f32),
            pltpu.VMEM((2, 8, M), f32),
            pltpu.VMEM((F // FC, B, FC), f32),
            pltpu.SMEM((NSLOT, M, D), bf16),
            pltpu.SemaphoreType.DMA((n_sems,)),
            pltpu.SemaphoreType.DMA((NSLOT,)),
            pltpu.SemaphoreType.DMA((NSLOT,)),
        ],
        compiler_params=pltpu.CompilerParams(
            vmem_limit_bytes=72 * 1024 * 1024,
            disable_semaphore_checks=True,
        ),
    )(x, B_w_r, A_c_kv, A_w_q, A_w_uk, A_w_uv, wo_t, B_w_gate, B_w_up, wd_t)
    return out.reshape(B, 1, M)
```

```python
import jax
import jax.numpy as jnp
from jax import lax
import jax.experimental.pallas as pl
import jax.experimental.pallas.tpu as pltpu

B, H, SK, D, M = 4, 32, 4096, 128, 576
DC = 4 * D
F = 4608
HH = 16
KC = 512
FC = 512
MS = 512
NS = 10
NSLOT = 4
WO_CHUNKS = (8, 6, 4, 2, 1, 1)
WDC = 3 * FC
EPS = 1e-5

f32 = jnp.float32
bf16 = jnp.bfloat16
NN = (((1,), (0,)), ((), ()))
NT = (((1,), (1,)), ((), ()))

assert NS + sum(WO_CHUNKS) == H and F % WDC == 0 and NSLOT <= NS <= 10


def _dot(a, b, dims):
    return lax.dot_general(a, b, dims, preferred_element_type=f32)


def _r(v):
    return v.astype(bf16).astype(f32)


def _kernel(x_hbm, wr_hbm, ckv_hbm, wq_hbm, wuk_hbm, wuv_hbm, wo_hbm, wg_hbm, wu_hbm, wd_hbm,
            o_hbm,
            x_v, wr_v, ckv_v, wq_v, wuk_v, wuv_v, wos_v, wolo_v, wohi_v, wg_v, wu_v, wd_v, o_v,
            rep_v, xexp_v, qabs_v, s_v, ctxc_v, ctxo_v, xg_v, h_v, stage_s,
            sems, hsems, ssems):
    n_sems = [0]

    def copy(src, dst):
        c = pltpu.make_async_copy(src, dst, sems.at[n_sems[0]])
        n_sems[0] += 1
        return c

    def h2s(j):
        return pltpu.make_async_copy(wo_hbm.at[j], stage_s.at[j % NSLOT], hsems.at[j % NSLOT])

    def s2v(j):
        return pltpu.make_async_copy(stage_s.at[j % NSLOT], wos_v.at[j], ssems.at[j % NSLOT])

    def smem_step(k):
        if k - 1 < NS:
            h2s(k - 1).wait()
            s2v(k - 1).start()
        if k + 1 < NS:
            if k + 1 >= NSLOT:
                s2v(k + 1 - NSLOT).wait()
            h2s(k + 1).start()

    c_wq = copy(wq_hbm, wq_v)
    c_x = copy(x_hbm, x_v)
    c_wr = copy(wr_hbm, wr_v)
    c_wuk = copy(wuk_hbm, wuk_v)
    c_ckv = [copy(ckv_hbm.at[b], ckv_v.at[b]) for b in range(B)]
    c_wuv = copy(wuv_hbm, wuv_v)
    c_wg = copy(wg_hbm, wg_v)
    c_wu = copy(wu_hbm, wu_v)
    c_wd = [copy(wd_hbm.at[:, pl.ds(i * WDC, WDC)], wd_v.at[i]) for i in range(F // WDC)]
    c_wo_hi = copy(wo_hbm.at[pl.ds(NS, H - NS), pl.ds(MS, M - MS)], wohi_v)
    c_wo = []
    h0 = 0
    for n in WO_CHUNKS:
        c_wo.append(copy(wo_hbm.at[pl.ds(NS + h0, n), pl.ds(0, MS)], wolo_v.at[pl.ds(h0, n)]))
        h0 += n
    c_out = copy(o_v, o_hbm)

    c_wq.start()
    c_x.start()
    c_wr.start()
    h2s(0).start()
    h2s(1).start()
    for c in [c_wuk] + c_ckv + [c_wuv, c_wg, c_wu] + c_wd + [c_wo_hi] + c_wo:
        c.start()

    def rep_body(t, carry):
        row = lax.broadcasted_iota(jnp.int32, (128, 256), 0)
        col = lax.broadcasted_iota(jnp.int32, (128, 256), 1) + t * 256
        rep_v[t] = jnp.where((col >> 4) == row, 1.0, 0.0).astype(bf16)
        return carry
    lax.fori_loop(0, 8, rep_body, 0)

    head_mask = ((lax.broadcasted_iota(jnp.int32, (B * HH, 256), 0) & (HH - 1))
                 == (lax.broadcasted_iota(jnp.int32, (B * HH, 256), 1) & (HH - 1)))

    smem_step(1)
    c_x.wait()
    c_wr.wait()
    x = x_v[...].astype(f32)
    mean = jnp.mean(x, axis=-1, keepdims=True)
    var = jnp.mean((x - mean) * (x - mean), axis=-1, keepdims=True)
    std = _r(jnp.sqrt(_r(_r(var) + EPS)))
    xn_b = (_r(x - _r(mean)) / std).astype(bf16)
    xn = xn_b.astype(f32)
    r = jnp.sum(xn * wr_v[...].astype(f32).reshape(1, M), axis=-1, keepdims=True)
    r_sel = _r(jax.nn.sigmoid(_r(r)))

    for j in range(5):
        w = 128 if j < 4 else M - 512
        xj = xn_b[:, 128 * j:128 * j + w]
        for t in range(w // 16):
            xr = _dot(xj, rep_v[t, 0:w, :], NN)
            xb = jnp.concatenate(
                [jnp.broadcast_to(xr[b:b + 1, :], (HH, 256)) for b in range(B)], axis=0)
            xexp_v[8 * j + t] = jnp.where(head_mask, xb, 0.0).astype(bf16)

    c_wq.wait()

    def q_body(t, carry):
        q0, q1 = carry
        lhs = xexp_v[t]
        m0 = pl.multiple_of(t * 16, 16)
        w0 = wq_v[pl.ds(m0, 16), 0:HH, :].reshape(256, D)
        w1 = wq_v[pl.ds(m0, 16), HH:H, :].reshape(256, D)
        return q0 + _dot(lhs, w0, NN), q1 + _dot(lhs, w1, NN)
    zero_q = jnp.zeros((B * HH, D), f32)
    q0, q1 = lax.fori_loop(0, M // 16, q_body, (zero_q, zero_q), unroll=4)
    scale = D ** -0.5
    qs = [(q0 * scale).astype(bf16), (q1 * scale).astype(bf16)]

    smem_step(2)
    c_wuk.wait()

    def qa_body(j, carry):
        for half in range(2):
            acc = jnp.zeros((B * HH, 128), f32)
            for t in range(8):
                c0 = pl.multiple_of(j * 128 + t * 16, 16)
                w = wuk_v[pl.ds(c0, 16), half * HH:(half + 1) * HH, :].reshape(256, D)
                allpairs = _dot(qs[half], w, NT)
                own = jnp.where(head_mask, allpairs, 0.0).astype(bf16)
                acc = acc + _dot(own, rep_v[t], NT)
            acc = acc.astype(bf16)
            for b in range(B):
                qabs_v[j, b, half * HH:(half + 1) * HH, :] = acc[b * HH:(b + 1) * HH, :]
        return carry
    lax.fori_loop(0, DC // 128, qa_body, 0)

    def attend(b):
        qa = jnp.concatenate([qabs_v[j, b] for j in range(DC // 128)], axis=1)

        def score_body(i, mx):
            k0 = pl.multiple_of(i * KC, KC)
            s = _dot(qa, ckv_v[b, pl.ds(k0, KC), :], NT)
            s_v[i] = s
            for u in range(KC // 128):
                mx = jnp.maximum(mx, s[:, u * 128:(u + 1) * 128])
            return mx
        mx = lax.fori_loop(0, SK // KC, score_body, jnp.full((H, 128), -jnp.inf, f32))
        row_max = jnp.max(mx, axis=-1, keepdims=True)

        def pv_body(i, carry):
            acc, den = carry
            k0 = pl.multiple_of(i * KC, KC)
            p = jnp.exp(s_v[i] - row_max)
            for u in range(KC // 128):
                den = den + p[:, u * 128:(u + 1) * 128]
            return acc + _dot(p.astype(bf16), ckv_v[b, pl.ds(k0, KC), :], NN), den
        acc, den = lax.fori_loop(0, SK // KC, pv_body,
                                 (jnp.zeros((H, DC), f32), jnp.zeros((H, 128), f32)))
        cc = (acc / jnp.sum(den, axis=-1, keepdims=True)).astype(bf16)
        for j in range(DC // 128):
            ctxc_v[j, b] = cc[:, j * 128:(j + 1) * 128]

    for b in range(B):
        smem_step(3 + b)
        c_ckv[b].wait()
        attend(b)

    smem_step(7)
    c_wuv.wait()

    def v_body(j, carry):
        out = []
        for half in range(2):
            acc = carry[half]
            lhs = jnp.concatenate(
                [ctxc_v[j, b, half * HH:(half + 1) * HH, :] for b in range(B)], axis=0)
            for t in range(8):
                c0 = pl.multiple_of(j * 128 + t * 16, 16)
                rep = _dot(lhs, rep_v[t], NN)
                own = jnp.where(head_mask, rep, 0.0).astype(bf16)
                w = wuv_v[pl.ds(c0, 16), half * HH:(half + 1) * HH, :].reshape(256, D)
                acc = acc + _dot(own, w, NN)
            out.append(acc)
        return tuple(out)
    ctx_halves = lax.fori_loop(0, DC // 128, v_body, (zero_q, zero_q))

    prow = lax.broadcasted_iota(jnp.int32, (8 * HH, B * HH), 0)
    pcol = lax.broadcasted_iota(jnp.int32, (8 * HH, B * HH), 1)
    perm = jnp.where(((prow >> 3) == (pcol & (HH - 1))) & ((prow & 7) == (pcol >> 4)),
                     1.0, 0.0).astype(bf16)
    for half, ctx in enumerate(ctx_halves):
        slabs = _dot(perm, ctx.astype(bf16), NN)
        for hh in range(HH):
            ctxo_v[half * HH + hh] = slabs[8 * hh:8 * hh + 8, :]

    smem_step(8)
    c_wg.wait()

    def gate_body(i, carry):
        c0 = pl.multiple_of(i * FC, FC)
        g = _r(_dot(xn_b, wg_v[:, pl.ds(c0, FC)], NN))
        h_v[i] = _r(g * jax.nn.sigmoid(g))
        return carry
    lax.fori_loop(0, F // FC, gate_body, 0)

    smem_step(9)
    c_wu.wait()

    def up_body(i, carry):
        c0 = pl.multiple_of(i * FC, FC)
        h_v[i] = h_v[i] * _r(_dot(xn_b, wu_v[:, pl.ds(c0, FC)], NN))
        return carry
    lax.fori_loop(0, F // FC, up_body, 0)
    smem_step(10)

    def out_proj(w_ref, i0, n, head0):
        lhs = jnp.concatenate([ctxo_v[head0 + i0 + i] for i in range(n)], axis=1).astype(bf16)
        w = jnp.concatenate([w_ref[i0 + i] for i in range(n)], axis=1)
        return _dot(lhs, w, NT)

    y = jnp.zeros((B, M), f32)
    for idx, c in enumerate(c_wd):
        if idx == len(c_wd) - 1:
            for j in range(NS - NSLOT, NS):
                s2v(j).wait()
            s = out_proj(wos_v, 0, NS, 0)
        c.wait()

        def down_body(i, y, idx=idx):
            c0 = pl.multiple_of(i * FC, FC)
            return y + _dot(h_v[idx * (WDC // FC) + i].astype(bf16),
                            wd_v[idx, :, pl.ds(c0, FC)], NT)
        y = lax.fori_loop(0, WDC // FC, down_body, y)
    z = _r(xn + _r(_r(y) * r_sel))
    gate = _r(z * jax.nn.sigmoid(z))

    xg_v[...] = jnp.zeros(xg_v.shape, f32)
    xg_v[0, 0:B, :] = x
    xg_v[1, 0:B, :] = gate

    c_wo_hi.wait()
    s_hi = s[:, MS:M] + out_proj(wohi_v, 0, H - NS, NS)
    o_v[:, MS:M] = (xg_v[0, :, MS:M] + s_hi * xg_v[1, :, MS:M])[0:B, :].astype(bf16)

    s = s[:, 0:MS]
    h0 = 0
    for n, c in zip(WO_CHUNKS[:-1], c_wo[:-1]):
        c.wait()
        s = s + out_proj(wolo_v, h0, n, NS)
        h0 += n
    gate_lo = xg_v[1, :, 0:MS]
    base = xg_v[0, :, 0:MS] + s * gate_lo
    c_wo[-1].wait()
    o_v[:, 0:MS] = (base + out_proj(wolo_v, h0, WO_CHUNKS[-1], NS) * gate_lo)[0:B, :].astype(bf16)

    c_out.start()
    c_out.wait()


@jax.jit
def pallas_recurrent_scan__compressed_kv_cla__moe_arch_mod__decode_kernel(
    A_x: jax.Array,
    A_c_kv: jax.Array,
    A_w_q: jax.Array,
    A_w_uk: jax.Array,
    A_w_uv: jax.Array,
    A_w_o: jax.Array,
    B_x: jax.Array,
    B_w_r: jax.Array,
    B_w_gate: jax.Array,
    B_w_up: jax.Array,
    B_w_down: jax.Array,
):
    del B_x
    x = A_x.reshape(B, M)
    wo_t = jnp.transpose(A_w_o, (0, 2, 1))
    wd_t = B_w_down.T
    hbm = pl.BlockSpec(memory_space=pl.ANY)
    n_sems = 4 + B + 3 + F // WDC + 1 + len(WO_CHUNKS) + 1
    out = pl.pallas_call(
        _kernel,
        out_shape=jax.ShapeDtypeStruct((B, M), bf16),
        in_specs=[hbm] * 10,
        out_specs=hbm,
        scratch_shapes=[
            pltpu.VMEM((B, M), bf16),
            pltpu.VMEM((M,), bf16),
            pltpu.VMEM((B, SK, DC), bf16),
            pltpu.VMEM((M, H, D), bf16),
            pltpu.VMEM((DC, H, D), bf16),
            pltpu.VMEM((DC, H, D), bf16),
            pltpu.VMEM((NS, M, D), bf16),
            pltpu.VMEM((H - NS, MS, D), bf16),
            pltpu.VMEM((H - NS, M - MS, D), bf16),
            pltpu.VMEM((M, F), bf16),
            pltpu.VMEM((M, F), bf16),
            pltpu.VMEM((F // WDC, M, WDC), bf16),
            pltpu.VMEM((B, M), bf16),
            pltpu.VMEM((8, 128, 256), bf16),
            pltpu.VMEM((M // 16, B * HH, 256), bf16),
            pltpu.VMEM((DC // 128, B, H, 128), bf16),
            pltpu.VMEM((SK // KC, H, KC), f32),
            pltpu.VMEM((DC // 128, B, H, 128), bf16),
            pltpu.VMEM((H, 8, D), f32),
            pltpu.VMEM((2, 8, M), f32),
            pltpu.VMEM((F // FC, B, FC), f32),
            pltpu.SMEM((NSLOT, M, D), bf16),
            pltpu.SemaphoreType.DMA((n_sems,)),
            pltpu.SemaphoreType.DMA((NSLOT,)),
            pltpu.SemaphoreType.DMA((NSLOT,)),
        ],
        compiler_params=pltpu.CompilerParams(
            vmem_limit_bytes=72 * 1024 * 1024,
            disable_semaphore_checks=True,
        ),
    )(x, B_w_r, A_c_kv, A_w_q, A_w_uk, A_w_uv, wo_t, B_w_gate, B_w_up, wd_t)
    return out.reshape(B, 1, M)
```

```python
import jax
import jax.numpy as jnp
from jax import lax
import jax.experimental.pallas as pl
import jax.experimental.pallas.tpu as pltpu

B, H, SK, D, M = 4, 32, 4096, 128, 576
DC = 4 * D
F = 4608
HH = 16
KC = 512
FC = 512
MS = 512
NS = 10
NSLOT = 4
WO_CHUNKS = (8, 6, 4, 2, 1, 1)
WD_ROWS = ((0, 256), (256, 256), (512, 64))
EPS = 1e-5

f32 = jnp.float32
bf16 = jnp.bfloat16
NN = (((1,), (0,)), ((), ()))
NT = (((1,), (1,)), ((), ()))

assert NS + sum(WO_CHUNKS) == H and NSLOT <= NS <= 10


def _dot(a, b, dims):
    return lax.dot_general(a, b, dims, preferred_element_type=f32)


def _r(v):
    return v.astype(bf16).astype(f32)


def _kernel(x_hbm, wr_hbm, ckv_hbm, wq_hbm, wuk_hbm, wuv_hbm, wo_hbm, wg_hbm, wu_hbm, wd_hbm,
            o_hbm,
            x_v, wr_v, ckv_v, wq_v, wuk_v, wuv_v, wos_v, wolo_v, wohi_v, wg_v, wu_v, wd_v, o_v,
            rep_v, xexp_v, qabs_v, s_v, ctxc_v, ctxo_v, xg_v, h_v, stage_s,
            sems, hsems, ssems):
    n_sems = [0]

    def copy(src, dst):
        c = pltpu.make_async_copy(src, dst, sems.at[n_sems[0]])
        n_sems[0] += 1
        return c

    def h2s(j):
        return pltpu.make_async_copy(wo_hbm.at[j], stage_s.at[j % NSLOT], hsems.at[j % NSLOT])

    def s2v(j):
        return pltpu.make_async_copy(stage_s.at[j % NSLOT], wos_v.at[j], ssems.at[j % NSLOT])

    def smem_step(k):
        if k - 1 < NS:
            h2s(k - 1).wait()
            s2v(k - 1).start()
        if k + 1 < NS:
            if k + 1 >= NSLOT:
                s2v(k + 1 - NSLOT).wait()
            h2s(k + 1).start()

    c_wq = copy(wq_hbm, wq_v)
    c_x = copy(x_hbm, x_v)
    c_wr = copy(wr_hbm, wr_v)
    c_wuk = copy(wuk_hbm, wuk_v)
    c_ckv = [copy(ckv_hbm.at[b], ckv_v.at[b]) for b in range(B)]
    c_wuv = copy(wuv_hbm, wuv_v)
    c_wg = copy(wg_hbm, wg_v)
    c_wu = copy(wu_hbm, wu_v)
    c_wd = [copy(wd_hbm.at[pl.ds(r0, n)], wd_v.at[pl.ds(r0, n)]) for r0, n in WD_ROWS]
    c_wo_hi = copy(wo_hbm.at[pl.ds(NS, H - NS), pl.ds(MS, M - MS)], wohi_v)
    c_wo = []
    h0 = 0
    for n in WO_CHUNKS:
        c_wo.append(copy(wo_hbm.at[pl.ds(NS + h0, n), pl.ds(0, MS)], wolo_v.at[pl.ds(h0, n)]))
        h0 += n
    c_out = copy(o_v, o_hbm)

    c_wq.start()
    c_x.start()
    c_wr.start()
    h2s(0).start()
    h2s(1).start()
    for c in [c_wuk] + c_ckv + [c_wuv, c_wg, c_wu] + c_wd + [c_wo_hi] + c_wo:
        c.start()

    def rep_body(t, carry):
        row = lax.broadcasted_iota(jnp.int32, (128, 256), 0)
        col = lax.broadcasted_iota(jnp.int32, (128, 256), 1) + t * 256
        rep_v[t] = jnp.where((col >> 4) == row, 1.0, 0.0).astype(bf16)
        return carry
    lax.fori_loop(0, 8, rep_body, 0)

    head_mask = ((lax.broadcasted_iota(jnp.int32, (B * HH, 256), 0) & (HH - 1))
                 == (lax.broadcasted_iota(jnp.int32, (B * HH, 256), 1) & (HH - 1)))

    smem_step(1)
    c_x.wait()
    c_wr.wait()
    x = x_v[...].astype(f32)
    mean = jnp.mean(x, axis=-1, keepdims=True)
    var = jnp.mean((x - mean) * (x - mean), axis=-1, keepdims=True)
    std = _r(jnp.sqrt(_r(_r(var) + EPS)))
    xn_b = (_r(x - _r(mean)) / std).astype(bf16)
    xn = xn_b.astype(f32)
    r = jnp.sum(xn * wr_v[...].astype(f32).reshape(1, M), axis=-1, keepdims=True)
    r_sel = _r(jax.nn.sigmoid(_r(r)))

    for j in range(5):
        w = 128 if j < 4 else M - 512
        xj = xn_b[:, 128 * j:128 * j + w]
        for t in range(w // 16):
            xr = _dot(xj, rep_v[t, 0:w, :], NN)
            xb = jnp.concatenate(
                [jnp.broadcast_to(xr[b:b + 1, :], (HH, 256)) for b in range(B)], axis=0)
            xexp_v[8 * j + t] = jnp.where(head_mask, xb, 0.0).astype(bf16)

    c_wq.wait()

    def q_body(t, carry):
        q0, q1 = carry
        lhs = xexp_v[t]
        m0 = pl.multiple_of(t * 16, 16)
        w0 = wq_v[pl.ds(m0, 16), 0:HH, :].reshape(256, D)
        w1 = wq_v[pl.ds(m0, 16), HH:H, :].reshape(256, D)
        return q0 + _dot(lhs, w0, NN), q1 + _dot(lhs, w1, NN)
    zero_q = jnp.zeros((B * HH, D), f32)
    q0, q1 = lax.fori_loop(0, M // 16, q_body, (zero_q, zero_q), unroll=4)
    scale = D ** -0.5
    qs = [(q0 * scale).astype(bf16), (q1 * scale).astype(bf16)]

    smem_step(2)
    c_wuk.wait()

    def qa_body(j, carry):
        for half in range(2):
            acc = jnp.zeros((B * HH, 128), f32)
            for t in range(8):
                c0 = pl.multiple_of(j * 128 + t * 16, 16)
                w = wuk_v[pl.ds(c0, 16), half * HH:(half + 1) * HH, :].reshape(256, D)
                allpairs = _dot(qs[half], w, NT)
                own = jnp.where(head_mask, allpairs, 0.0).astype(bf16)
                acc = acc + _dot(own, rep_v[t], NT)
            acc = acc.astype(bf16)
            for b in range(B):
                qabs_v[j, b, half * HH:(half + 1) * HH, :] = acc[b * HH:(b + 1) * HH, :]
        return carry
    lax.fori_loop(0, DC // 128, qa_body, 0)

    def attend(b):
        qa = jnp.concatenate([qabs_v[j, b] for j in range(DC // 128)], axis=1)

        def score_body(i, mx):
            k0 = pl.multiple_of(i * KC, KC)
            s = _dot(qa, ckv_v[b, pl.ds(k0, KC), :], NT)
            s_v[i] = s
            for u in range(KC // 128):
                mx = jnp.maximum(mx, s[:, u * 128:(u + 1) * 128])
            return mx
        mx = lax.fori_loop(0, SK // KC, score_body, jnp.full((H, 128), -jnp.inf, f32))
        row_max = jnp.max(mx, axis=-1, keepdims=True)

        def pv_body(i, carry):
            acc, den = carry
            k0 = pl.multiple_of(i * KC, KC)
            p = jnp.exp(s_v[i] - row_max)
            for u in range(KC // 128):
                den = den + p[:, u * 128:(u + 1) * 128]
            return acc + _dot(p.astype(bf16), ckv_v[b, pl.ds(k0, KC), :], NN), den
        acc, den = lax.fori_loop(0, SK // KC, pv_body,
                                 (jnp.zeros((H, DC), f32), jnp.zeros((H, 128), f32)))
        cc = (acc / jnp.sum(den, axis=-1, keepdims=True)).astype(bf16)
        for j in range(DC // 128):
            ctxc_v[j, b] = cc[:, j * 128:(j + 1) * 128]

    for b in range(B):
        smem_step(3 + b)
        c_ckv[b].wait()
        attend(b)

    smem_step(7)
    c_wuv.wait()

    def v_body(j, carry):
        out = []
        for half in range(2):
            acc = carry[half]
            lhs = jnp.concatenate(
                [ctxc_v[j, b, half * HH:(half + 1) * HH, :] for b in range(B)], axis=0)
            for t in range(8):
                c0 = pl.multiple_of(j * 128 + t * 16, 16)
                rep = _dot(lhs, rep_v[t], NN)
                own = jnp.where(head_mask, rep, 0.0).astype(bf16)
                w = wuv_v[pl.ds(c0, 16), half * HH:(half + 1) * HH, :].reshape(256, D)
                acc = acc + _dot(own, w, NN)
            out.append(acc)
        return tuple(out)
    ctx_halves = lax.fori_loop(0, DC // 128, v_body, (zero_q, zero_q))

    prow = lax.broadcasted_iota(jnp.int32, (8 * HH, B * HH), 0)
    pcol = lax.broadcasted_iota(jnp.int32, (8 * HH, B * HH), 1)
    perm = jnp.where(((prow >> 3) == (pcol & (HH - 1))) & ((prow & 7) == (pcol >> 4)),
                     1.0, 0.0).astype(bf16)
    for half, ctx in enumerate(ctx_halves):
        slabs = _dot(perm, ctx.astype(bf16), NN)
        for hh in range(HH):
            ctxo_v[half * HH + hh] = slabs[8 * hh:8 * hh + 8, :]

    smem_step(8)
    c_wg.wait()

    def gate_body(i, carry):
        c0 = pl.multiple_of(i * FC, FC)
        g = _r(_dot(xn_b, wg_v[:, pl.ds(c0, FC)], NN))
        h_v[i] = _r(g * jax.nn.sigmoid(g))
        return carry
    lax.fori_loop(0, F // FC, gate_body, 0)

    smem_step(9)
    c_wu.wait()

    def up_body(i, carry):
        c0 = pl.multiple_of(i * FC, FC)
        h_v[i] = h_v[i] * _r(_dot(xn_b, wu_v[:, pl.ds(c0, FC)], NN))
        return carry
    lax.fori_loop(0, F // FC, up_body, 0)
    smem_step(10)

    y_parts = []
    for c, (r0, n) in zip(c_wd, WD_ROWS):
        c.wait()

        def down_body(i, y, r0=r0, n=n):
            c0 = pl.multiple_of(i * FC, FC)
            return y + _dot(h_v[i].astype(bf16), wd_v[r0:r0 + n, pl.ds(c0, FC)], NT)
        y_parts.append(lax.fori_loop(0, F // FC, down_body, jnp.zeros((B, n), f32), unroll=3))
    y = jnp.concatenate(y_parts, axis=1)
    z = _r(xn + _r(_r(y) * r_sel))
    gate = _r(z * jax.nn.sigmoid(z))

    xg_v[...] = jnp.zeros(xg_v.shape, f32)
    xg_v[0, 0:B, :] = x
    xg_v[1, 0:B, :] = gate

    def out_proj(w_ref, i0, n, head0):
        lhs = jnp.concatenate([ctxo_v[head0 + i0 + i] for i in range(n)], axis=1).astype(bf16)
        w = jnp.concatenate([w_ref[i0 + i] for i in range(n)], axis=1)
        return _dot(lhs, w, NT)

    for j in range(NS - NSLOT, NS):
        s2v(j).wait()
    s = out_proj(wos_v, 0, NS, 0)

    c_wo_hi.wait()
    s_hi = s[:, MS:M] + out_proj(wohi_v, 0, H - NS, NS)
    o_v[:, MS:M] = (xg_v[0, :, MS:M] + s_hi * xg_v[1, :, MS:M])[0:B, :].astype(bf16)

    s = s[:, 0:MS]
    h0 = 0
    for n, c in zip(WO_CHUNKS[:-1], c_wo[:-1]):
        c.wait()
        s = s + out_proj(wolo_v, h0, n, NS)
        h0 += n
    gate_lo = xg_v[1, :, 0:MS]
    base = xg_v[0, :, 0:MS] + s * gate_lo
    c_wo[-1].wait()
    o_v[:, 0:MS] = (base + out_proj(wolo_v, h0, WO_CHUNKS[-1], NS) * gate_lo)[0:B, :].astype(bf16)

    c_out.start()
    c_out.wait()


@jax.jit
def pallas_recurrent_scan__compressed_kv_cla__moe_arch_mod__decode_kernel(
    A_x: jax.Array,
    A_c_kv: jax.Array,
    A_w_q: jax.Array,
    A_w_uk: jax.Array,
    A_w_uv: jax.Array,
    A_w_o: jax.Array,
    B_x: jax.Array,
    B_w_r: jax.Array,
    B_w_gate: jax.Array,
    B_w_up: jax.Array,
    B_w_down: jax.Array,
):
    del B_x
    x = A_x.reshape(B, M)
    wo_t = jnp.transpose(A_w_o, (0, 2, 1))
    wd_t = B_w_down.T
    hbm = pl.BlockSpec(memory_space=pl.ANY)
    n_sems = 4 + B + 3 + len(WD_ROWS) + 1 + len(WO_CHUNKS) + 1
    out = pl.pallas_call(
        _kernel,
        out_shape=jax.ShapeDtypeStruct((B, M), bf16),
        in_specs=[hbm] * 10,
        out_specs=hbm,
        scratch_shapes=[
            pltpu.VMEM((B, M), bf16),
            pltpu.VMEM((M,), bf16),
            pltpu.VMEM((B, SK, DC), bf16),
            pltpu.VMEM((M, H, D), bf16),
            pltpu.VMEM((DC, H, D), bf16),
            pltpu.VMEM((DC, H, D), bf16),
            pltpu.VMEM((NS, M, D), bf16),
            pltpu.VMEM((H - NS, MS, D), bf16),
            pltpu.VMEM((H - NS, M - MS, D), bf16),
            pltpu.VMEM((M, F), bf16),
            pltpu.VMEM((M, F), bf16),
            pltpu.VMEM((M, F), bf16),
            pltpu.VMEM((B, M), bf16),
            pltpu.VMEM((8, 128, 256), bf16),
            pltpu.VMEM((M // 16, B * HH, 256), bf16),
            pltpu.VMEM((DC // 128, B, H, 128), bf16),
            pltpu.VMEM((SK // KC, H, KC), f32),
            pltpu.VMEM((DC // 128, B, H, 128), bf16),
            pltpu.VMEM((H, 8, D), f32),
            pltpu.VMEM((2, 8, M), f32),
            pltpu.VMEM((F // FC, B, FC), f32),
            pltpu.SMEM((NSLOT, M, D), bf16),
            pltpu.SemaphoreType.DMA((n_sems,)),
            pltpu.SemaphoreType.DMA((NSLOT,)),
            pltpu.SemaphoreType.DMA((NSLOT,)),
        ],
        compiler_params=pltpu.CompilerParams(
            vmem_limit_bytes=72 * 1024 * 1024,
            disable_semaphore_checks=True,
        ),
    )(x, B_w_r, A_c_kv, A_w_q, A_w_uk, A_w_uv, wo_t, B_w_gate, B_w_up, wd_t)
    return out.reshape(B, 1, M)
```
